```python
import os as _os
_os.environ.setdefault("JAX_PLATFORMS", "cpu")
import jax
import jax.numpy as jnp

def _softmax(x, axis=-1):
    return jax.nn.softmax(x, axis=axis)
def _gelu(x):
    return jax.nn.gelu(x, approximate=True)
def _silu(x):
    return jax.nn.silu(x)
def _sigmoid(x):
    return jax.nn.sigmoid(x)
def _layernorm(x, axis=-1, eps=1e-5):
    m = jnp.mean(x, axis=axis, keepdims=True)
    v = jnp.var(x, axis=axis, keepdims=True)
    return (x - m) / jnp.sqrt(v + eps)
def _scatter_add(tgt, idx, src, axis=0):
    return tgt.at[idx].add(src)
def _segment_sum(src, seg, n):
    return jax.ops.segment_sum(src, seg, n)
class _Rng:
    def __init__(self, key):
        self._k = key
    def _next(self):
        self._k, sub = jax.random.split(self._k)
        return sub
    def normal(self, shape):
        return jax.random.normal(self._next(), shape, dtype=jnp.bfloat16)
    def randint(self, lo, hi, shape):
        return jax.random.randint(self._next(), shape, lo, hi, dtype=jnp.int32)
    def uniform(self, shape, lo=0.0, hi=1.0):
        return jax.random.uniform(self._next(), shape, jnp.bfloat16, lo, hi)
    def permutation(self, n):
        return jax.random.permutation(self._next(), n)


kernel_name = 'gated_mix__softmax_full_mha__dense_activation_relu__prompt'

def setup_inputs():
    _rng = _Rng(jax.random.key(int.from_bytes(__import__("os").urandom(4), "little")))
    _w = (lambda a: (lambda t: t.astype(jnp.bfloat16) if jnp.issubdtype(t.dtype, jnp.floating) else t)(jnp.asarray(a)))
    def _A_setup():
        B, S, D = 1, 2048, 640
        return {
            "x": _w((lambda *s: _rng.normal(s) * 0.05)(B, S, D)),
            "wqkv": _w((lambda *s: _rng.normal(s) * 0.8)(D, 3 * D)),
            "wo": _w((lambda *s: _rng.normal(s) * 0.05)(D, D)),
        }
    _A_in = _A_setup()

    def _B_setup():
        B, S, D, Dff = 1, 2048, 640, 1536
        return {
            "x": _w((lambda *s: _rng.normal(s) * 0.05)(B, S, D)),
            "w1": _w((lambda *s: _rng.normal(s) * 0.05)(D, Dff)),
            "w2": _w((lambda *s: _rng.normal(s) * 0.05)(Dff, D)),
        }
    _B_in = _B_setup()

    return {
        "A_x": _A_in["x"],
        "A_wqkv": _A_in["wqkv"],
        "A_wo": _A_in["wo"],
        "B_x": _B_in["x"],
        "B_w1": _B_in["w1"],
        "B_w2": _B_in["w2"],
        "gate_w": _w((lambda *s: _rng.normal(s) * 0.05)(640) * 16.0),
    }

def reference(A_x, A_wqkv, A_wo, B_x, B_w1, B_w2, gate_w):
    def _A_ref(x, wqkv, wo):
        B, S, D = x.shape
        H = 32; Dh = D // H
        qkv = (lambda x, *d: x.transpose(*d))((x @ wqkv).reshape(B, S, 3, H, Dh), 2, 0, 3, 1, 4)
        q, k, v = qkv[0], qkv[1], qkv[2]
        scale = Dh ** -0.5
        scores = jnp.einsum("bhqd,bhkd->bhqk", q, k) * scale
        p = _softmax(scores, axis=-1)
        o = jnp.einsum("bhqk,bhkd->bhqd", p, v)
        return (lambda x, *d: x.transpose(*d))(o, 0, 2, 1, 3).reshape(B, S, D) @ wo

    def _B_ref(x, w1, w2):
        h = jnp.einsum("bsd,df->bsf", x, w1)
        zero = jnp.zeros_like(h)
        h = jnp.maximum(h, zero)
        return jnp.einsum("bsf,fd->bsd", h, w2)

    x = A_x
    g = _sigmoid((x * gate_w).sum(-1, keepdims=True))
    a = _A_ref(x, A_wqkv, A_wo)
    b = _B_ref(x, B_w1, B_w2)
    return g * a + (1 - g) * b
```

```python
import functools, math
import jax, jax.numpy as jnp, numpy as np
from jax import lax
from jax.experimental import pallas as pl
from jax.experimental.pallas import tpu as pltpu

S, D, H, DH, DFF = 2048, 640, 32, 20, 1536
NTILE = D // 128
F32, BF16 = jnp.float32, jnp.bfloat16
NT_DIMS = (((1,), (1,)), ((), ()))
TN_DIMS = (((0,), (0,)), ((), ()))
QSCALE = float(DH ** -0.5 * math.log2(math.e))

def make(BQ=512, CK=256, VROWS=32, flags=None):
    NQB = S // BQ
    NCK = S // CK
    VDT = BF16 if VROWS == 32 else F32
    def kernel(x_ref, wqkv_ref, wo_ref, w1_ref, w2_ref, gw_ref, o_ref,
               k_s, vt_s, qt_s, s_s, ot_s, wqt_s):
        i = pl.program_id(0)

        @pl.when(i == 0)
        def _():
            wqt_s[...] = wqkv_ref[:, 0:D].T
            wvt = wqkv_ref[:, 2 * D:3 * D].T
            RB = 512
            lane = lax.broadcasted_iota(jnp.int32, (RB, 128), 1)
            sub = lax.broadcasted_iota(jnp.int32, (24, RB), 0)
            for r in range(S // RB):
                xr = x_ref[r * RB:(r + 1) * RB, :]
                k = jnp.dot(xr, wqkv_ref[:, D:2 * D], preferred_element_type=F32)
                for j in range(NTILE):
                    k_s[j, r * RB:(r + 1) * RB, :] = k[:, j * 128:(j + 1) * 128].astype(BF16)
                for j in range(NTILE - 1):
                    t = jnp.where(lane < 64, k[:, (j + 1) * 128:(j + 2) * 128], k[:, j * 128:(j + 1) * 128])
                    k_s[NTILE + j, r * RB:(r + 1) * RB, :] = t.astype(BF16)
                vt = lax.dot_general(wvt, xr, NT_DIMS, preferred_element_type=F32)
                for h in range(H):
                    lo = (h * DH // 8) * 8
                    w = vt[lo:lo + 24, :]
                    one_row = 20 if h % 2 == 0 else 0
                    w = jnp.where(sub == one_row, 1.0, w)
                    if VROWS == 32:
                        w = jnp.concatenate([w, jnp.zeros((8, RB), F32)], axis=0)
                    vt_s[h, :, r * RB:(r + 1) * RB] = w.astype(VDT)

        xq = x_ref[pl.ds(pl.multiple_of(i * BQ, BQ), BQ), :]
        qt = lax.dot_general(wqt_s[...], xq, NT_DIMS, preferred_element_type=F32) * QSCALE
        row = lax.broadcasted_iota(jnp.int32, (128, BQ), 0)
        for j in range(NTILE):
            qt_s[j] = qt[j * 128:(j + 1) * 128]
        for j in range(NTILE - 1):
            qt_s[NTILE + j] = jnp.where(row < 64, qt[(j + 1) * 128:(j + 2) * 128], qt[j * 128:(j + 1) * 128])

        def head_q(h):
            lo = h * DH
            j = lo // 128
            off = lo % 128
            t = jnp.where(off > 128 - DH, NTILE + j, j)
            msk = ((row - off) & 127) < DH
            return t, jnp.where(msk, qt_s[t], 0.0).astype(BF16)

        def step(h, m, do_qk, do_pv):
            if do_qk:
                t, qm = head_q(h + 1)
            acc = None
            mn = None
            for c in range(NCK):
                ks = slice(c * CK, (c + 1) * CK)
                if do_pv:
                    p = jnp.exp2(s_s[ks, :] - m).astype(BF16)
                    d = jnp.dot(vt_s[h, :, ks], p, preferred_element_type=F32)
                    acc = d if acc is None else acc + d
                if do_qk:
                    s = jnp.dot(k_s[t, ks, :], qm, preferred_element_type=F32)
                    s_s[ks, :] = s
                    mc = jnp.max(s.reshape(CK // 8, 8, BQ), axis=0)
                    mn = mc if mn is None else jnp.maximum(mn, mc)
            if do_qk:
                mn = jnp.max(mn, axis=0, keepdims=True)
            return mn, acc

        def finish(hp, a0, a1):
            o0 = a0[0:24] / a0[20:21]
            o1 = a1[0:24] / a1[0:1]
            sub = lax.broadcasted_iota(jnp.int32, (8, BQ), 0)
            mid = jnp.where(sub < 4, o0[16:24], o1[0:8])
            ot_s[pl.ds(pl.multiple_of(hp * 40, 8), 40), :] = jnp.concatenate([o0[0:16], mid, o1[8:24]], axis=0)

        m0, _ = step(-1, None, True, False)

        def body(hp, m):
            m, a0 = step(2 * hp, m, True, True)
            m, a1 = step(2 * hp + 1, m, True, True)
            finish(hp, a0, a1)
            return m

        m = lax.fori_loop(0, H // 2 - 1, body, m0)
        m, a0 = step(H - 2, m, True, True)
        _, a1 = step(H - 1, m, False, True)
        finish(H // 2 - 1, a0, a1)

        a = lax.dot_general(ot_s[...].astype(BF16), wo_ref[...], TN_DIMS, preferred_element_type=F32)
        hh = jnp.maximum(jnp.dot(xq, w1_ref[...], preferred_element_type=F32), 0.0).astype(BF16)
        b = jnp.dot(hh, w2_ref[...], preferred_element_type=F32)
        g = jax.nn.sigmoid(jnp.sum(xq.astype(F32) * gw_ref[...].astype(F32), axis=-1, keepdims=True))
        o_ref[...] = (g * a + (1.0 - g) * b).astype(o_ref.dtype)

    def full(shape):
        return pl.BlockSpec(shape, lambda i: (0,) * len(shape), pipeline_mode=pl.Buffered(1))

    @jax.jit
    def pallas_gated_mix__softmax_full_mha__dense_activation_relu__prompt_kernel(A_x, A_wqkv, A_wo, B_x, B_w1, B_w2, gate_w):
        out = pl.pallas_call(
            kernel, grid=(NQB,),
            in_specs=[full((S, D)), full((D, 3 * D)), full((D, D)), full((D, DFF)), full((DFF, D)), full((1, D))],
            out_specs=pl.BlockSpec((BQ, D), lambda i: (i, 0)),
            out_shape=jax.ShapeDtypeStruct((S, D), BF16),
            scratch_shapes=[pltpu.VMEM((2 * NTILE - 1, S, 128), BF16), pltpu.VMEM((H, VROWS, S), VDT),
                            pltpu.VMEM((2 * NTILE - 1, 128, BQ), F32), pltpu.VMEM((S, BQ), F32),
                            pltpu.VMEM((D, BQ), F32), pltpu.VMEM((D, D), BF16)],
            compiler_params=pltpu.CompilerParams(dimension_semantics=("arbitrary",), vmem_limit_bytes=100 * 2**20, flags=flags),
        )(A_x.reshape(S, D), A_wqkv, A_wo, B_w1, B_w2, gate_w.reshape(1, D))
        return out.reshape(1, S, D)
    return pallas_gated_mix__softmax_full_mha__dense_activation_relu__prompt_kernel


pallas_gated_mix__softmax_full_mha__dense_activation_relu__prompt_kernel = make(BQ=512,CK=256)
```

```python
import math

import jax
import jax.numpy as jnp
from jax import lax
from jax.experimental import pallas as pl
from jax.experimental.pallas import tpu as pltpu

S, D, H, DH, DFF = 2048, 640, 32, 20, 1536
F32, BF16 = jnp.float32, jnp.bfloat16
NTILE = D // 128
QSCALE = float(DH ** -0.5 * math.log2(math.e))

BQ = 512
CK = 128
UNROLL = 8
RB = 256
KT = 3
WB = 256
VROWS = 24
NQB, NCK, NX = S // BQ, S // CK, S // RB
NIT = NQB * H // UNROLL
HB, HD = BQ // 2, D // 2

L, M, R = slice(0, 256), slice(256, 384), slice(384, 640)
LM, MR = slice(0, 384), slice(256, 640)
N1, N2 = slice(0, DFF // 2), slice(DFF // 2, DFF)


def _add(p, q):
    return (p.astype(F32) + q.astype(F32)).astype(BF16)


def _sub(p, q):
    return (p.astype(F32) - q.astype(F32)).astype(BF16)


def _cat(p, q):
    return jnp.concatenate([p, q], axis=1)


def _dot(p, q):
    return lax.dot_general(p, q, (((1,), (0,)), ((), ())), preferred_element_type=F32)


def _dot_nt(p, q):
    return lax.dot_general(p, q, (((1,), (1,)), ((), ())), preferred_element_type=F32)


def _dot_tn(p, q):
    return lax.dot_general(p, q, (((0,), (0,)), ((), ())), preferred_element_type=F32)


def _rows(start, n):
    if isinstance(start, int):
        return pl.ds(start, n)
    return pl.ds(pl.multiple_of(start, n), n)


def _kernel(x_hbm, wqkv_hbm, wo_hbm, w1_hbm, w2_hbm, gw_hbm, o_hbm,
            x_s, wq_s, wk_s, wv_s, wo_s, w1_s, w2_s, gw_s,
            k_s, vt_s, qt_s, s_s, acc_s, ot_s, a_s, out_s, ua, u1, u2,
            xsem, wsem, osem):
    def cp_x(r):
        rows = _rows(r * RB, RB)
        return pltpu.make_async_copy(x_hbm.at[rows, :], x_s.at[rows, :], xsem.at[r])

    def cp_out(u):
        rows = _rows(u * HB, HB)
        return pltpu.make_async_copy(out_s.at[rows, :], o_hbm.at[rows, :], osem.at[u])

    cp_wq = pltpu.make_async_copy(wqkv_hbm.at[:, 0:D], wq_s, wsem.at[0])
    cp_wk = pltpu.make_async_copy(wqkv_hbm.at[:, D:2 * D], wk_s, wsem.at[1])
    cp_wv = pltpu.make_async_copy(wqkv_hbm.at[:, 2 * D:3 * D], wv_s, wsem.at[2])
    cp_late = [
        pltpu.make_async_copy(w1_hbm, w1_s, wsem.at[3]),
        pltpu.make_async_copy(w2_hbm, w2_s, wsem.at[4]),
        pltpu.make_async_copy(wo_hbm, wo_s, wsem.at[5]),
        pltpu.make_async_copy(gw_hbm, gw_s, wsem.at[6]),
    ]

    cp_wk.start()
    cp_x(0).start()
    cp_x(1).start()
    s_s[1] = jnp.zeros((S, BQ), F32)
    cp_wk.wait()
    for r in range(2, NX):
        cp_x(r).start()
    cp_wv.start()
    cp_wq.start()

    lane = lax.broadcasted_iota(jnp.int32, (RB, 128), 1)

    def k_proj(r):
        k = _dot(x_s[_rows(r * RB, RB), :], wk_s[...])
        tiles = [k[:, j * 128:(j + 1) * 128] for j in range(NTILE)]
        tiles += [jnp.where(lane < 64, tiles[j + 1], tiles[j]) for j in range(NTILE - 1)]
        for j, t in enumerate(tiles):
            k_s[j, _rows(r * (RB // 2), RB // 2), :] = pltpu.bitcast(t.astype(BF16), jnp.uint32)

    @pl.loop(0, NX - KT)
    def _(r):
        cp_x(r).wait()
        k_proj(r)

    for r in range(NX - KT, NX):
        cp_x(r).wait()
    cp_wv.wait()
    cp_wq.wait()
    for e, w_s in enumerate((wq_s, wv_s)):
        w = w_s[...].T
        a1, a2 = w[:HD], w[HD:]
        rs = slice(e * HD, (e + 1) * HD)
        ua[0, rs, L] = _add(a1[:, L], a2[:, R])
        ua[1, rs, L] = _add(a2[:, L], a2[:, R])
        ua[2, rs] = a1[:, LM]
        ua[3, rs] = a2[:, MR]
        ua[4, rs, L] = _add(a1[:, L], a1[:, R])
        ua[5, rs] = _sub(a2[:, LM], a1[:, LM])
        ua[6, rs] = _sub(a1[:, MR], a2[:, MR])
    for r in range(NX - KT, NX):
        k_proj(r)

    vrow = lax.broadcasted_iota(jnp.int32, (VROWS, BQ), 0)
    row = lax.broadcasted_iota(jnp.int32, (128, BQ), 0)

    @pl.loop(0, NQB)
    def _(i):
        @pl.when(i == 1)
        def _():
            for cp in cp_late:
                cp.start()

        xr = x_s[_rows(i * BQ, BQ), :]
        x1, x2 = xr[:HB], xr[HB:]
        m5 = _dot_nt(ua[4, :, L], x2[:, R])
        m3 = _dot_nt(ua[2], _cat(_sub(x2[:, L], x2[:, R]), x2[:, M]))
        c12 = m3 + m5
        m2 = _dot_nt(ua[1, :, L], x1[:, L])
        m4 = _dot_nt(ua[3], _cat(x1[:, M], _sub(x1[:, R], x1[:, L])))
        c21 = m2 + m4
        m1 = _dot_nt(ua[0, :, L], _add(x1[:, L], x2[:, R]))
        m7 = _dot_nt(ua[6], _cat(x1[:, M], _add(x1[:, R], x2[:, R])))
        c11 = (m4 - m5) + m1 + m7
        m6 = _dot_nt(ua[5], _cat(_add(x1[:, L], x2[:, L]), x2[:, M]))
        c22 = (m3 - m2) + m1 + m6
        c1, c2 = _cat(c11, c12), _cat(c21, c22)
        qt = jnp.concatenate([c1[:HD], c2[:HD]], axis=0) * QSCALE
        vt = jnp.concatenate([c1[HD:], c2[HD:]], axis=0)
        tiles = [qt[j * 128:(j + 1) * 128] for j in range(NTILE)]
        tiles += [jnp.where(row < 64, tiles[j + 1], tiles[j]) for j in range(NTILE - 1)]
        for j, t in enumerate(tiles):
            qt_s[i, j] = t.astype(BF16)
        for h in range(H):
            lo = (h * DH // 8) * 8
            vt_s[i, h] = jnp.where(vrow == (0 if h % 2 else DH), 1.0, vt[lo:lo + VROWS, :])

    for cp in cp_late:
        cp.wait()

    def ffn_weight_sums(it, e):
        def part(base, n):
            return _rows(base + it * (n // NIT), n // NIT)

        top, mid, bot = part(0, 256), part(256, 128), part(384, 256)
        ra, rb = part(0, DFF // 2), part(DFF // 2, DFF // 2)
        if e == 0:
            u1[0, top] = _add(w1_s[top, N1], w1_s[bot, N2])
            u2[0, ra, L] = _add(w2_s[ra, L], w2_s[rb, R])
        elif e == 1:
            u1[1, top] = _sub(w1_s[top, N2], w1_s[bot, N2])
            u1[1, mid] = w1_s[mid, N2]
            u2[1, ra] = _sub(w2_s[ra, MR], w2_s[rb, MR])
        elif e == 2:
            u1[2, part(128, 256)] = _sub(w1_s[bot, N1], w1_s[top, N1])
            u1[2, part(0, 128)] = w1_s[mid, N1]
            u2[2, ra] = _sub(w2_s[rb, LM], w2_s[ra, LM])
        elif e == 3:
            u1[3, top] = _add(w1_s[top, N1], w1_s[top, N2])
            u1[3, mid] = w1_s[mid, N2]
            u2[3, ra, L] = _add(w2_s[ra, L], w2_s[ra, R])
        else:
            u1[4, part(128, 256)] = _add(w1_s[bot, N1], w1_s[bot, N2])
            u1[4, part(0, 128)] = w1_s[mid, N1]
            u2[4, ra, L] = _add(w2_s[rb, L], w2_s[rb, R])
        return (u1[0, top, 0:128].astype(F32) + u2[0, top, 0:128].astype(F32))[0:1]

    def softmax_pv(n, m, src, c):
        p = jnp.exp2(src[c * CK:(c + 1) * CK, :] - m).astype(BF16)
        kb, ko = divmod(c * CK, BQ)
        return _dot(vt_s[kb, n & (H - 1), :, ko:ko + CK], p)

    def step(n, m, src, dst):
        lo = (n & (H - 1)) * DH
        off = lo & 127
        t = jnp.where(off > 128 - DH, NTILE + (lo >> 7), lo >> 7)
        qm = jnp.where(((row - off) & 127) < DH, qt_s[n >> 5, t], 0.0)
        acc = mx = None
        for c in range(NCK):
            s = _dot(pltpu.bitcast(k_s[t, c * CK // 2:(c + 1) * CK // 2, :], BF16), qm)
            dst[c * CK:(c + 1) * CK, :] = s
            mc = jnp.max(s.reshape(CK // 8, 8, BQ), axis=0)
            mx = mc if c == 0 else jnp.maximum(mx, mc)
            d = softmax_pv(n - 1, m, src, c)
            acc = d if c == 0 else acc + d
        acc_s[n] = acc
        return jnp.max(mx, axis=0, keepdims=True)

    bufs = (s_s.at[0], s_s.at[1])

    def attention(it, m):
        for u in range(UNROLL):
            if 1 <= u <= 5:
                tie = ffn_weight_sums(it, u - 1)
                m = jnp.where(it < 0, jnp.concatenate([tie] * (BQ // 128), axis=1), m)
            m = step(it * UNROLL + u, m, bufs[(u + 1) % 2], bufs[u % 2])
        return m

    m_last = lax.fori_loop(0, NIT, attention, jnp.zeros((1, BQ), F32))

    sub8 = lax.broadcasted_iota(jnp.int32, (8, BQ), 0)
    per = NCK * WB // (2 * BQ)
    last = None
    for i in range(NQB):
        for hp in range(H // 2):
            n = i * H + 2 * hp
            a0 = acc_s[n + 1]
            a1 = acc_s[n + 2] if n + 2 < NQB * H else last
            o0 = a0 / a0[DH:DH + 1]
            o1 = a1 / a1[0:1]
            ot_s[i, hp * 2 * DH:(hp + 1) * 2 * DH, :] = jnp.concatenate(
                [o0[0:16], jnp.where(sub8 < 4, o0[16:24], o1[0:8]), o1[8:24]], axis=0)
        for e in range(BQ // WB):
            k = i * (BQ // WB) + e
            for c in range(k * per, min((k + 1) * per, NCK)):
                d = softmax_pv(NQB * H - 1, m_last, bufs[1], c)
                last = d if c == 0 else last + d
            a_s[k * WB:(k + 1) * WB, :] = _dot_tn(
                ot_s[i, :, e * WB:(e + 1) * WB].astype(BF16), wo_s[...])

    @pl.loop(0, NQB)
    def _(i):
        xq = x_s[_rows(i * BQ, BQ), :]
        gw = gw_s[...].astype(F32).reshape(1, D)
        g = jax.nn.sigmoid(jnp.sum(xq.astype(F32) * gw, axis=-1, keepdims=True))
        x1, x2 = xq[:HB], xq[HB:]
        m3 = _dot(x1[:, LM], u1[1])
        m5 = _dot(_add(x1[:, L], x1[:, R]), w1_s[R, N2])
        h12 = jnp.maximum(m3 + m5, 0.0)
        m4 = _dot(x2[:, MR], u1[2])
        m2 = _dot(_add(x2[:, L], x2[:, R]), w1_s[L, N1])
        h21 = jnp.maximum(m2 + m4, 0.0)
        m1 = _dot(_add(x1[:, L], x2[:, R]), u1[0, L])
        m7 = _dot(_sub(x1[:, MR], x2[:, MR]), u1[4])
        h11 = jnp.maximum((m4 - m5) + m1 + m7, 0.0)
        m6 = _dot(_sub(x2[:, LM], x1[:, LM]), u1[3])
        h22 = jnp.maximum((m3 - m2) + m1 + m6, 0.0)

        def mix(e, b):
            rows = _rows(i * BQ + e * HB, HB)
            ge = g[e * HB:(e + 1) * HB]
            out_s[rows, :] = (ge * a_s[rows, :] + (1.0 - ge) * b).astype(BF16)
            cp_out(2 * i + e).start()

        m3 = _dot(h11.astype(BF16), u2[1])
        m5 = _dot(_add(h11, h12), w2_s[N2, MR])
        m4 = _dot(h22.astype(BF16), u2[2])
        m1 = _dot(_add(h11, h22), u2[0, :, L])
        m7 = _dot(_sub(h12, h22), u2[4, :, L])
        mix(0, _cat((m4[:, :256] - m5[:, 128:]) + m1 + m7, m3 + m5))
        m2 = _dot(_add(h21, h22), w2_s[N1, LM])
        m6 = _dot(_sub(h21, h11), u2[3, :, L])
        mix(1, _cat(m2 + m4, (m3[:, 128:] + m1 - m2[:, :256]) + m6))

    for u in range(S // HB):
        cp_out(u).wait()


@jax.jit
def pallas_gated_mix__softmax_full_mha__dense_activation_relu__prompt_kernel(
    A_x: jax.Array,
    A_wqkv: jax.Array,
    A_wo: jax.Array,
    B_x: jax.Array,
    B_w1: jax.Array,
    B_w2: jax.Array,
    gate_w: jax.Array,
):
    del B_x
    hbm = pl.BlockSpec(memory_space=pl.ANY)
    out = pl.pallas_call(
        _kernel,
        in_specs=[hbm] * 6,
        out_specs=hbm,
        out_shape=jax.ShapeDtypeStruct((S, D), BF16),
        scratch_shapes=[
            pltpu.VMEM((S, D), BF16),
            pltpu.VMEM((D, D), BF16),
            pltpu.VMEM((D, D), BF16),
            pltpu.VMEM((D, D), BF16),
            pltpu.VMEM((D, D), BF16),
            pltpu.VMEM((D, DFF), BF16),
            pltpu.VMEM((DFF, D), BF16),
            pltpu.VMEM((D,), BF16),
            pltpu.VMEM((2 * NTILE - 1, S // 2, 128), jnp.uint32),
            pltpu.VMEM((NQB, H, VROWS, BQ), F32),
            pltpu.VMEM((NQB, 2 * NTILE - 1, 128, BQ), BF16),
            pltpu.VMEM((2, S, BQ), F32),
            pltpu.VMEM((NQB * H, VROWS, BQ), F32),
            pltpu.VMEM((NQB, D, BQ), F32),
            pltpu.VMEM((S, D), F32),
            pltpu.VMEM((S, D), BF16),
            pltpu.VMEM((7, D, 384), BF16),
            pltpu.VMEM((5, 384, DFF // 2), BF16),
            pltpu.VMEM((5, DFF // 2, 384), BF16),
            pltpu.SemaphoreType.DMA((NX,)),
            pltpu.SemaphoreType.DMA((7,)),
            pltpu.SemaphoreType.DMA((S // HB,)),
        ],
        compiler_params=pltpu.CompilerParams(vmem_limit_bytes=100 * 2**20),
    )(A_x.reshape(S, D), A_wqkv, A_wo, B_w1, B_w2, gate_w)
    return out.reshape(1, S, D)
```
